```python
import os as _os
_os.environ.setdefault("JAX_PLATFORMS", "cpu")
import jax
import jax.numpy as jnp

def _softmax(x, axis=-1):
    return jax.nn.softmax(x, axis=axis)
def _gelu(x):
    return jax.nn.gelu(x, approximate=True)
def _silu(x):
    return jax.nn.silu(x)
def _sigmoid(x):
    return jax.nn.sigmoid(x)
def _layernorm(x, axis=-1, eps=1e-5):
    m = jnp.mean(x, axis=axis, keepdims=True)
    v = jnp.var(x, axis=axis, keepdims=True)
    return (x - m) / jnp.sqrt(v + eps)
def _scatter_add(tgt, idx, src, axis=0):
    return tgt.at[idx].add(src)
def _segment_sum(src, seg, n):
    return jax.ops.segment_sum(src, seg, n)
class _Rng:
    def __init__(self, key):
        self._k = key
    def _next(self):
        self._k, sub = jax.random.split(self._k)
        return sub
    def normal(self, shape):
        return jax.random.normal(self._next(), shape, dtype=jnp.bfloat16)
    def randint(self, lo, hi, shape):
        return jax.random.randint(self._next(), shape, lo, hi, dtype=jnp.int32)
    def uniform(self, shape, lo=0.0, hi=1.0):
        return jax.random.uniform(self._next(), shape, jnp.bfloat16, lo, hi)
    def permutation(self, n):
        return jax.random.permutation(self._next(), n)


kernel_name = 'interleave_layers__sliding_block_cached__mixer_channel_mlp__decode'

def setup_inputs():
    _rng = _Rng(jax.random.key(int.from_bytes(__import__("os").urandom(4), "little")))
    _w = (lambda a: (lambda t: t.astype(jnp.bfloat16) if jnp.issubdtype(t.dtype, jnp.floating) else t)(jnp.asarray(a)))
    def _A_setup():
        B, Sq, D = 8, 1, 1024
        Hq, Hkv, Sk, Dh = 32, 4, 4096, 128
        assert Hq % Hkv == 0, (Hq, Hkv)
        return {
            "x": _w((lambda *s: _rng.normal(s) * 0.05)(B, Sq, D)),
            "k_cache": _w((lambda *s: _rng.normal(s) * 1.6)(B, Hkv, Sk, Dh)),
            "v_cache": _w((lambda *s: _rng.normal(s) * 0.8)(B, Hkv, Sk, Dh)),
            "wq": _w((lambda *s: _rng.normal(s) * 1.6)(D, Hq * Dh) * (D ** -0.5)),
            "wo": _w((lambda *s: _rng.normal(s) * 0.8)(Hq * Dh, D) * ((Hq * Dh) ** -0.5)),
        }
    _A_in = _A_setup()

    def _B_setup():
        B, S, D, F = 8, 1, 1024, 3584
        return {
            "x": _w((lambda *s: _rng.normal(s) * 0.05)(B, S, D)),
            "w1": _w((lambda *s: _rng.normal(s) * 0.4)(D, F) * (D ** -0.5)),
            "b1": _w((lambda *s: _rng.normal(s) * 0.4)(F)),
            "w2": _w((lambda *s: _rng.normal(s) * 0.4)(F, D) * (F ** -0.5)),
            "b2": _w((lambda *s: _rng.normal(s) * 0.1)(D)),
        }
    _B_in = _B_setup()

    return {
        "A_x": _A_in["x"],
        "A_k_cache": _A_in["k_cache"],
        "A_v_cache": _A_in["v_cache"],
        "A_wq": _A_in["wq"],
        "A_wo": _A_in["wo"],
        "B_x": _B_in["x"],
        "B_w1": _B_in["w1"],
        "B_b1": _B_in["b1"],
        "B_w2": _B_in["w2"],
        "B_b2": _B_in["b2"],
    }

def reference(A_x, A_k_cache, A_v_cache, A_wq, A_wo, B_x, B_w1, B_b1, B_w2, B_b2):
    def _A_ref(x, k_cache, v_cache, wq, wo):
        B, Sq, D = x.shape
        Hq, Dh = 32, 128
        Hkv, Sk = k_cache.shape[1], k_cache.shape[2]
        W = min(4096, max(256, Sk // 4))
        rep = Hq // Hkv
        q = (lambda x, *d: x.transpose(*d))((x @ wq).reshape(B, Sq, Hq, Dh), 0, 2, 1, 3)
        k = jnp.repeat(k_cache[:, :, Sk - W:, :], rep, axis=1)
        v = jnp.repeat(v_cache[:, :, Sk - W:, :], rep, axis=1)
        scores = jnp.einsum("bhqd,bhkd->bhqk", q, k) * (Dh ** -0.5)
        p = _softmax(scores, axis=-1)
        o = jnp.einsum("bhqk,bhkd->bhqd", p, v)
        return (lambda x, *d: x.transpose(*d))(o, 0, 2, 1, 3).reshape(B, Sq, Hq * Dh) @ wo

    def _B_ref(x, w1, b1, w2, b2):
        y = _layernorm(x, axis=-1)
        h = _gelu(jnp.einsum("bsd,df->bsf", y, w1) + b1)
        return jnp.einsum("bsf,fd->bsd", h, w2) + b2

    x = A_x
    x = x + _A_ref(_layernorm(x, axis=-1), A_k_cache, A_v_cache, A_wq, A_wo)
    x = x + _B_ref(_layernorm(x, axis=-1), B_w1, B_b1, B_w2, B_b2)
    x = x + _A_ref(_layernorm(x, axis=-1), A_k_cache, A_v_cache, A_wq, A_wo)
    x = x + _B_ref(_layernorm(x, axis=-1), B_w1, B_b1, B_w2, B_b2)
    return x
```

```python
import functools

import jax
import jax.numpy as jnp
import numpy as np
from jax import lax
import jax.experimental.pallas as pl
import jax.experimental.pallas.tpu as pltpu

BF = jnp.bfloat16
F32 = jnp.float32
EPS = 1e-5
HQ, DH = 32, 128


def _tile_view(w):
    K, N = w.shape
    w = w.reshape(K // 16, 2, 8, N // 256, 2, 128).transpose(0, 1, 3, 4, 2, 5)
    return w.reshape(K // 16, 2, N // 256, 16, 128)


def _lhs_pair(cols):
    lane = lax.broadcasted_iota(jnp.int32, (8, 128), 1)
    even = (lane & 8) == 0
    p0, p1 = [], []
    for x in cols:
        xe = jnp.where(even, x, 0.0)
        xo = jnp.where(even, 0.0, x)
        p0.append(jnp.concatenate([xe, pltpu.roll(xe, 8, 1)], axis=0).astype(BF))
        p1.append(jnp.concatenate([pltpu.roll(xo, 120, 1), xo], axis=0).astype(BF))
    return jnp.concatenate(p0, axis=1), jnp.concatenate(p1, axis=1)


def _mm(lhs, w_ref, k0, n):
    kk = lhs[0].shape[1]
    r = None
    for p in range(2):
        w = w_ref[pl.ds(k0 * 8, kk // 16), p, n].reshape(kk, 128)
        d = jnp.dot(lhs[p], w, preferred_element_type=F32)
        r = d if r is None else r + d
    return r


def _rowsum(cols):
    t = cols[0]
    for c in cols[1:]:
        t = t + c
    return jnp.sum(t, axis=1, keepdims=True)


def _stats(cols):
    n = 128 * len(cols)
    m = _rowsum(cols) * (1.0 / n)
    d = [c - m for c in cols]
    v = _rowsum([c * c for c in d]) * (1.0 / n)
    return m, lax.rsqrt(v + EPS), d


def _ln(cols):
    _, r, d = _stats(cols)
    return [c * r for c in d]


def _gelu(x):
    c = np.float32(np.sqrt(2.0 / np.pi))
    return 0.5 * x * (1.0 + jnp.tanh(c * (x + 0.044715 * (x * x * x))))


def _rnd(x):
    return x.astype(BF).astype(F32)


def make(tail_rows=1024, tail_cols=(2, 1, 1), main_split=(1792, 768)):
    B, D, G, W, F = 8, 1024, 4, 1024, 3584
    ND, NQ, NF = D // 128, HQ * DH // 128, F // 128
    assert sum(main_split) + tail_rows == F

    def kernel(x_h, k_h, v_h, wq_h, wo_h, w1_h, b1_h, w2_h, b2_h, o_ref,
               x_v, k_v, v_v, wq_v, wo_v, w1_v, b1_v, w2_v, b2_v, kt_v, qs_v, os_v, cq_v, c1_v, sems):
        Sk = k_h.shape[2]
        cps = []

        def dma(src, dst):
            c = pltpu.make_async_copy(src, dst, sems.at[len(cps)])
            cps.append(c)
            c.start()
            return c

        c_wq = dma(wq_h, wq_v)
        c_x = dma(x_h, x_v)
        c_k = dma(k_h.at[:, :, pl.ds(Sk - W, W), :], k_v)
        c_v = dma(v_h.at[:, :, pl.ds(Sk - W, W), :], v_v)
        c_wo = dma(wo_h, wo_v)
        c_b1 = dma(b1_h, b1_v)
        c_b2 = dma(b2_h, b2_v)
        c_w1 = dma(w1_h, w1_v)
        c_w2 = []
        r0 = 0
        for r in main_split:
            c_w2.append((r0, r, dma(w2_h.at[pl.ds(r0 // 16, r // 16)], w2_v.at[pl.ds(r0 // 16, r // 16)])))
            r0 += r
        c_w2t = []
        n0 = 0
        for n in tail_cols:
            sl = (pl.ds(r0 // 16, tail_rows // 16), slice(None), pl.ds(n0, n))
            c_w2t.append((n0, n, dma(w2_h.at[sl], w2_v.at[sl])))
            n0 += n

        lane = lax.broadcasted_iota(jnp.int32, (16, D), 1)
        row = lax.broadcasted_iota(jnp.int32, (16, D), 0)
        ones = jnp.where((lane & 8) == (row & 8), 1.0, 0.0).astype(BF)

        def with_colsum(cols, w_ref, cs_ref, nn):
            l0, l1 = _lhs_pair(cols)
            lhs = (jnp.concatenate([l0, ones], axis=0), jnp.concatenate([l1, ones], axis=0))
            out = []
            for n in range(nn // 2):
                r = _mm(lhs, w_ref, 0, n)
                out += [r[0:8], r[8:16]]
                cs_ref[pl.ds(16 * n, 16), :] = r[16:32]
            return out

        def put_q(h, q):
            qs_v[pl.ds(8 * h, 8), :] = q

        def scores(g, bp):
            q = jnp.concatenate([qs_v[pl.ds(64 * g + 2 * bp + i, 8, stride=8), :] for i in range(2)], axis=0).astype(BF)
            s = []
            for i in range(2):
                kt = jnp.concatenate([kt_v[2 * bp + i, g, j] for j in range(W // 128)], axis=1)
                s.append(jnp.dot(q, kt, preferred_element_type=F32)[8 * i:8 * i + 8])
            s = jnp.concatenate(s, axis=0)
            m = jnp.max(s, axis=1, keepdims=True)
            e = jnp.exp(s - m)
            l = jnp.sum(e, axis=1, keepdims=True)
            return e.astype(BF), 1.0 / l

        def pv(g, bp, p, linv):
            for i in range(2):
                o = jnp.dot(p, v_v[2 * bp + i, g], preferred_element_type=F32)[8 * i:8 * i + 8]
                os_v[pl.ds(64 * g + 2 * bp + i, 8, stride=8), :] = o * linv[8 * i:8 * i + 8]

        def o_lhs(g):
            return _lhs_pair([os_v[pl.ds(64 * g + 8 * h, 8), :] for h in range(8)])

        scale = np.float32(DH ** -0.5)

        c_x.wait()
        x0f = x_v[...].astype(F32)
        x0 = [x0f[:, 128 * j:128 * j + 128] for j in range(ND)]
        y = _ln(x0)
        c_wq.wait()
        q = with_colsum(y, wq_v, cq_v, NQ)
        for h in range(NQ):
            put_q(h, _rnd(q[h]) * scale)
        c_k.wait()

        def tr_body(i, carry):
            b = i // G
            g = i % G
            for j in range(W // 128):
                kt_v[b, g, j] = k_v[b, g, pl.ds(128 * j, 128), :].T
            return carry

        lax.fori_loop(0, B * G, tr_body, 0)
        c_v.wait()
        for g in range(G):
            for bp in range(B // 2):
                p, linv = scores(g, bp)
                pv(g, bp, p, linv)
        c_wo.wait()
        acc = [None] * (ND // 2)
        for g in range(G):
            lhs = o_lhs(g)
            for n in range(ND // 2):
                r = _mm(lhs, wo_v, 8 * g, n)
                acc[n] = r if acc[n] is None else acc[n] + r
        x1 = []
        for n in range(ND // 2):
            x1 += [_rnd(x0[2 * n] + acc[n][0:8]), _rnd(x0[2 * n + 1] + acc[n][8:16])]
        y = _ln(_ln(x1))
        c_b1.wait()
        c_b2.wait()
        b1 = b1_v[...].astype(F32)
        b2 = b2_v[...].astype(F32)
        c_w1.wait()
        hp = with_colsum(y, w1_v, c1_v, NF)
        h = [_gelu(hp[j] + b1[j:j + 1]) for j in range(NF)]
        acc = [None] * (ND // 2)
        for (r0, r, c) in c_w2:
            lhs = _lhs_pair(h[r0 // 128:(r0 + r) // 128])
            c.wait()
            for n in range(ND // 2):
                t = _mm(lhs, w2_v, r0 // 128, n)
                acc[n] = t if acc[n] is None else acc[n] + t
        kt0 = (F - tail_rows) // 128
        lhs = _lhs_pair(h[kt0:])
        x2 = []
        qacc = [None] * (NQ // 2)
        for ci, (n0, nn, c) in enumerate(c_w2t):
            c.wait()
            for n in range(n0, n0 + nn):
                t = acc[n] + _mm(lhs, w2_v, kt0, n)
                for i in range(2):
                    j = 2 * n + i
                    x2.append(_rnd(x1[j] + (t[8 * i:8 * i + 8] + b2[j:j + 1])))
            xl = _lhs_pair(x2[2 * n0:])
            if ci == len(c_w2t) - 1:
                m, r, _ = _stats(x2)
                rs = r
            for n in range(NQ // 2):
                t = _mm(xl, wq_v, 2 * n0, n)
                qacc[n] = t if qacc[n] is None else qacc[n] + t
                if ci == len(c_w2t) - 1:
                    for i in range(2):
                        hh = 2 * n + i
                        qv = (qacc[n][8 * i:8 * i + 8] - m * cq_v[pl.ds(8 * hh, 8), :]) * rs
                        put_q(hh, _rnd(qv) * scale)

        acc = [None] * (ND // 2)

        def wo_block(g, ns):
            lhs = o_lhs(g)
            for n in ns:
                r = _mm(lhs, wo_v, 8 * g, n)
                acc[n] = r if acc[n] is None else acc[n] + r

        items = [(g, bp) for g in range(G) for bp in range(B // 2)]
        DEPTH = 2
        pend = []
        for it in items:
            pend.append((it, scores(*it)))
            if len(pend) > DEPTH:
                (g, bp), (p, linv) = pend.pop(0)
                pv(g, bp, p, linv)
        wo_block(0, range(ND // 2))
        for (g, bp), (p, linv) in pend:
            pv(g, bp, p, linv)
        for g in range(1, G):
            wo_block(g, range(ND // 2))
        x3 = []
        for n in range(ND // 2):
            x3 += [_rnd(x2[2 * n] + acc[n][0:8]), _rnd(x2[2 * n + 1] + acc[n][8:16])]
        m1, r1, d = _stats(x3)
        m2, r2, _ = _stats([c * r1 for c in d])
        a = r1 * r2
        cc = (m1 * r1 + m2) * r2
        HALF = ND // 2
        xa = _lhs_pair(x3[:HALF])
        xb = _lhs_pair(x3[HALF:])
        NPRE = 4
        pre = [_mm(xa, w1_v, 0, n) for n in range(NPRE)]
        h = []
        acc = [None] * (ND // 2)
        done = 0

        def w2_block(j0, j1):
            lhs = _lhs_pair(h[j0:j1])
            for n in range(ND // 2):
                t = _mm(lhs, w2_v, j0, n)
                acc[n] = t if acc[n] is None else acc[n] + t

        for n in range(NF // 2):
            t = pre[n] if n < NPRE else _mm(xa, w1_v, 0, n)
            t = t + _mm(xb, w1_v, HALF, n)
            for i in range(2):
                j = 2 * n + i
                h.append(_gelu(t[8 * i:8 * i + 8] * a - cc * c1_v[pl.ds(8 * j, 8), :] + b1[j:j + 1]))
        for j0 in range(0, NF, 4):
            w2_block(j0, j0 + 4)
        out = []
        for n in range(ND // 2):
            for i in range(2):
                j = 2 * n + i
                out.append(x3[j] + (acc[n][8 * i:8 * i + 8] + b2[j:j + 1]))
        o_ref[...] = jnp.concatenate(out, axis=1).astype(o_ref.dtype)

    def fn(A_x, A_k_cache, A_v_cache, A_wq, A_wo, B_x, B_w1, B_b1, B_w2, B_b2):
        any_ = pl.BlockSpec(memory_space=pl.ANY)
        wq, wo, w1, w2 = (_tile_view(w) for w in (A_wq, A_wo, B_w1, B_w2))
        out = pl.pallas_call(
            kernel,
            out_shape=jax.ShapeDtypeStruct((B, D), A_x.dtype),
            in_specs=[any_] * 9,
            scratch_shapes=[
                pltpu.VMEM((B, D), BF),
                pltpu.VMEM((B, G, W, DH), BF),
                pltpu.VMEM((B, G, W, DH), BF),
                pltpu.VMEM(wq.shape, BF),
                pltpu.VMEM(wo.shape, BF),
                pltpu.VMEM(w1.shape, BF),
                pltpu.VMEM((NF, 128), BF),
                pltpu.VMEM(w2.shape, BF),
                pltpu.VMEM((ND, 128), BF),
                pltpu.VMEM((B, G, W // 128, DH, 128), BF),
                pltpu.VMEM((HQ * B, DH), F32),
                pltpu.VMEM((HQ * B, DH), F32),
                pltpu.VMEM((NQ * 8, 128), F32),
                pltpu.VMEM((NF * 8, 128), F32),
                pltpu.SemaphoreType.DMA((8 + len(main_split) + len(tail_cols),)),
            ],
            compiler_params=pltpu.CompilerParams(
                vmem_limit_bytes=100 * 1024 * 1024, disable_semaphore_checks=True),
        )(A_x.reshape(B, D), A_k_cache, A_v_cache, wq, wo, w1, B_b1.reshape(NF, 128), w2, B_b2.reshape(ND, 128))
        return out.reshape(A_x.shape)

    return fn


@jax.jit
def pallas_interleave_layers__sliding_block_cached__mixer_channel_mlp__decode_kernel(
    A_x, A_k_cache, A_v_cache, A_wq, A_wo, B_x, B_w1, B_b1, B_w2, B_b2
):
    return make()(A_x, A_k_cache, A_v_cache, A_wq, A_wo, B_x, B_w1, B_b1, B_w2, B_b2)
```

```python
import jax
import jax.numpy as jnp
import numpy as np
from jax import lax
import jax.experimental.pallas as pl
import jax.experimental.pallas.tpu as pltpu

BF = jnp.bfloat16
F32 = jnp.float32
EPS = 1e-5
HQ, DH = 32, 128


def _tile_view(w):
    K, N = w.shape
    w = w.reshape(K // 16, 2, 8, N // 256, 2, 128).transpose(0, 1, 3, 4, 2, 5)
    return w.reshape(K // 16, 2, N // 256, 16, 128)


def _ld(ref, idx):
    w = ref.bitcast(jnp.int32)[idx]
    return pltpu.bitcast(w.reshape(-1, 128), BF)


def _lhs_pair(cols):
    lane = lax.broadcasted_iota(jnp.int32, (8, 128), 1)
    even = (lane & 8) == 0
    p0, p1 = [], []
    for x in cols:
        xe = jnp.where(even, x, 0.0)
        xo = jnp.where(even, 0.0, x)
        p0.append(jnp.concatenate([xe, pltpu.roll(xe, 8, 1)], axis=0).astype(BF))
        p1.append(jnp.concatenate([pltpu.roll(xo, 120, 1), xo], axis=0).astype(BF))
    return list(zip(p0, p1))


def _mm(lhs, w_ref, k0, n):
    kts = range(k0, k0 + len(lhs)) if isinstance(k0, int) else k0
    r = None
    for p in range(2):
        a, w = [t[p] for t in lhs], []
        if len(w_ref.shape) == 5:
            w += [_ld(w_ref, (pl.ds(k * 8, 8), p, n)) for k in kts]
        else:
            nn = w_ref.shape[0] // 128
            w += [_ld(w_ref, (pl.ds((k * 16 + p) * nn + n, 8, stride=2 * nn),)) for k in kts]
        d = jnp.dot(jnp.concatenate(a, axis=1), jnp.concatenate(w, axis=0), preferred_element_type=F32)
        r = d if r is None else r + d
    return r


def _rowsum(cols):
    t = cols[0]
    for c in cols[1:]:
        t = t + c
    return jnp.sum(t, axis=1, keepdims=True)


def _stats(cols):
    n = 128 * len(cols)
    m = _rowsum(cols) * (1.0 / n)
    d = [c - m for c in cols]
    v = _rowsum([c * c for c in d]) * (1.0 / n)
    return m, lax.rsqrt(v + EPS), d


def _ln(cols):
    _, r, d = _stats(cols)
    return [c * r for c in d]


def _gelu(x):
    c = np.float32(np.sqrt(2.0 / np.pi))
    return 0.5 * x * (1.0 + jnp.tanh(c * (x + 0.044715 * (x * x * x))))


def _rnd(x):
    return x.astype(BF).astype(F32)


def _add(acc, n, r):
    acc[n] = r if acc[n] is None else acc[n] + r


A8, B8, C4, T8 = (0, 4, 7, 11, 14, 18, 21, 25), (1, 5, 8, 12, 15, 19, 22, 26), (2, 9, 16, 23), (3, 6, 10, 13, 17, 20, 24, 27)
COLS = [[(A8, 0, 4)], [(B8, 0, 4)], [(C4, 0, 4), (T8, 0, 1)], [(T8, 1, 2)], [(T8, 2, 3)], [(T8, 3, 4)]]
D6, D3, D2 = (1, 6, 10, 15, 20, 24), (3, 13, 22), (8, 27)
R8, R9 = (0, 4, 7, 11, 14, 18, 21, 25), (2, 5, 9, 12, 16, 17, 19, 23, 26)
STAIR = [[(R8, 0, 4)], [(R9, 0, 4)], [(D3, 0, 2), (D2, 0, 1), (D6, 0, 3)], [(D2, 1, 4)], [(D3, 2, 4)], [(D6, 3, 4)]]


def make(plan=COLS, shift=32, lag=112, nocomp=False, probe=None, DEPTH=2, defer=8, VO=0, V2=0, NPRE=4, sa=4, so=2, s1=2, s2=1, first=1):
    B, D, G, W, F = 8, 1024, 4, 1024, 3584
    ND, NQ, NF = D // 128, HQ * DH // 128, F // 128
    S = 8

    def kernel(x_h, k_h, v_h, wq_h, wo_h, w1_h, b1_h, w2_h, b2_h, o_ref,
               x_v, k_v, v_v, wq_v, wo_v, w1_v, b1_v, w2_v, b2_v, kt_v, qs_v, os_v, cq_v, c1_v, lhs_v, acc_v,
               wof_v, w2f_v, xb_v, av_v, sems):
        Sk = k_h.shape[2]

        rounds, whole = [], []

        def streamed(n, h, v, idx, hidx=None):
            sem = sems.at[len(whole)]

            def issue(t):
                for s in range(S):
                    pltpu.make_async_copy(h.at[(hidx or idx)(s, t)], v.at[idx(s, t)], sem).start(priority=s % 2)

            rounds.append((n, issue))
            whole.append([v])
            return len(whole) - 1

        def kv_idx(off):
            return lambda s, t: (s, t >> 3, pl.ds(pl.multiple_of(off + (t & 7) * 128, 128), 128))

        g_wq = streamed(32, wq_h, wq_v, lambda s, t: (s * 8 + (t >> 2), (t >> 1) & 1, pl.ds((t & 1) * 8, 8)))
        g_k = streamed(32, k_h, k_v, kv_idx(0), kv_idx(Sk - W))
        g_v = streamed(32, v_h, v_v, kv_idx(0), kv_idx(Sk - W))
        g_wo = streamed(32, wo_h, wo_v, lambda s, t: (s * 32 + t,))
        g_w1 = streamed(28, w1_h, w1_v, lambda s, t: (pl.ds((s * 28 + t) * 8, 8),))
        ((kts0, _, _),) = plan[0]
        g_w2 = streamed(8, w2_h, w2_v, lambda s, t: (8 * kts0[s] + t,))
        whole[g_w2] = [w2_v.at[pl.ds(8 * k, 8)] for k in kts0]
        todo = []
        for stage in plan[1:]:
            whole.append([])
            for kts, n0, n1 in stage:
                per = max(1, 4 // (n1 - n0))
                whole[-1] += [w2_v.at[pl.ds(8 * k, 8), :, pl.ds(n0, n1 - n0)] for k in kts]
                todo += [((pl.ds(8 * k + i, per), slice(None), pl.ds(n0, n1 - n0)), len(whole) - 1)
                         for i in range(0, 8, per) for k in kts]
        head, last = todo[:len(todo) - shift], todo[len(todo) - shift:]
        q0, q1 = head[0::2], head[1::2] + last
        lead = len(q1) - len(q0)
        order = [(d, 1) for d in q1[:lead]] + [x for a, b in zip(q0, q1[lead:]) for x in ((a, 0), (b, 1))]
        for i in range(0, len(order), S):
            def issue(t, part=order[i:i + S]):
                for (idx, gi), prio in part:
                    pltpu.make_async_copy(w2_h.at[idx], w2_v.at[idx], sems.at[gi]).start(priority=prio)

            rounds.append((1, issue))
        starts = [int(v) for v in np.cumsum([0] + [r[0] for r in rounds])]
        pos = [0]

        def issue_to(hi, body=None, per=1):
            hi, done = min(hi, starts[-1]), 0
            for gi, (n, issue) in enumerate(rounds):
                a, b = max(pos[0], starts[gi]), min(hi, starts[gi + 1])
                if a >= b:
                    continue
                assert (b - a) % per == 0

                def step(t, issue=issue, t0=a - starts[gi], done=done):
                    for u in range(per):
                        issue(t0 + t * per + u)
                    if body is not None:
                        body(done + t)

                if n == 1:
                    step(0)
                else:
                    pl.loop(0, (b - a) // per)(step)
                done += (b - a) // per
            pos[0] = max(pos[0], hi)

        def overlapped(n, per=1):
            return lambda body: issue_to(pos[0] + n * per, body, per)

        def wait(gi):
            assert pos[0] >= (starts[gi + 1] if gi <= g_w2 else starts[-1])
            for v in whole[gi]:
                pltpu.make_async_copy(v, v, sems.at[gi]).wait()

        def landed(gi):
            issue_to(starts[gi + 1] + lag // S)
            wait(gi)

        small = [pltpu.make_async_copy(h, v, sems.at[len(whole) + i])
                 for i, (h, v) in enumerate(((x_h, x_v), (b1_h, b1_v), (b2_h, b2_v)))]
        issue_to(1)
        for c in small:
            c.start()

        if nocomp:
            issue_to(starts[-1])
            if probe is not None:
                if probe < 0:
                    wait(len(whole) + probe)
                pl.delay(10000)
            for c in small:
                c.wait()
            for gi in range(len(whole)):
                if probe is None or gi != len(whole) + probe:
                    wait(gi)
            o_ref[...] = x_v[...]
            return

        def stage_lhs(cols, k0=0, ones=False):
            lane = lax.broadcasted_iota(jnp.int32, (16, 128), 1)
            row = lax.broadcasted_iota(jnp.int32, (16, 128), 0)
            one = jnp.where((lane & 8) == (row & 8), 1.0, 0.0).astype(BF)
            for k, t in enumerate(_lhs_pair(cols)):
                for p in range(2):
                    lhs_v[k0 + k, p, pl.ds(0, 16), :] = t[p]
                    if ones:
                        lhs_v[k0 + k, p, pl.ds(16, 16), :] = one

        def staged(kts, m=16):
            return [tuple(lhs_v[k, p, pl.ds(0, m), :] for p in range(2)) for k in kts]

        def rows16(n):
            return pl.ds(pl.multiple_of(16 * n, 16), 16)

        def scores(g, bp):
            q = jnp.concatenate([qs_v[g, pl.ds(2 * bp + i, 8, stride=8), :] for i in range(2)], axis=0).astype(BF)
            s = []
            for i in range(2):
                kt = jnp.concatenate([_ld(kt_v, (2 * bp + i, g, j)) for j in range(W // 128)], axis=1)
                s.append(jnp.dot(q, kt, preferred_element_type=F32)[8 * i:8 * i + 8])
            s = jnp.concatenate(s, axis=0)
            m = jnp.max(s, axis=1, keepdims=True)
            e = jnp.exp(s - m)
            l = jnp.sum(e, axis=1, keepdims=True)
            return e.astype(BF), 1.0 / l

        def pv(g, bp, p, linv):
            for i in range(2):
                o = jnp.dot(p, _ld(v_v, (2 * bp + i, g)), preferred_element_type=F32)[8 * i:8 * i + 8]
                os_v[g, pl.ds(2 * bp + i, 8, stride=8), :] = o * linv[8 * i:8 * i + 8]

        def put_q(n, q):
            qs_v[n >> 2, rows16(n & 3), :] = _rnd(q) * np.float32(DH ** -0.5)

        def halves(acc):
            return [a[8 * i:8 * i + 8] for a in acc for i in range(2)]

        landed(g_wq)
        for c in small:
            c.wait()
        x0f = x_v[...].astype(F32)
        x0 = [x0f[:, 128 * j:128 * j + 128] for j in range(ND)]
        stage_lhs(_ln(x0), ones=True)
        acc_v[pl.ds(0, 8 * ND), :] = jnp.concatenate(x0, axis=0)

        @overlapped(NQ // 2)
        def _(n):
            r = _mm(staged(range(ND), 32), wq_v, 0, n)
            cq_v[rows16(n), :] = r[16:32]
            put_q(n, r[0:16])

        landed(g_k)

        @overlapped(B * G)
        def _(i):
            b, g = i >> 2, i & 3
            for j in range(W // 128):
                kt_v[b, g, j] = k_v[b, g, pl.ds(128 * j, 128), :].T

        landed(g_v)

        @overlapped(G * B // 2, 2)
        def _(i):
            g, bp = i >> 2, i & 3
            pv(g, bp, *scores(g, bp))

        @pl.loop(0, G)
        def _(g):
            stage_lhs([os_v[g, pl.ds(8 * h, 8), :] for h in range(8)], 8 * g)

        landed(g_wo)

        @overlapped(G * ND // 2)
        def _(i):
            g, n = i >> 2, i & 3
            kts = [8 * g + h for h in range(8)]
            acc_v[rows16(n), :] += _mm(staged(kts), wo_v, kts, n)

        if VO:
            @pl.loop(0, 8 * VO)
            def _(i):
                wof_v[i] = wo_v[i].astype(F32)

        x1 = [_rnd(acc_v[pl.ds(8 * j, 8), :]) for j in range(ND)]
        stage_lhs(_ln(_ln(x1)), ones=True)
        landed(g_w1)
        b1 = b1_v[...].astype(F32)
        b2 = b2_v[...].astype(F32)

        for i in range(2):
            @pl.loop(i * NF // 4, (i + 1) * NF // 4)
            def _(n):
                r = _mm(staged(range(ND), 32), w1_v, 0, n)
                c1_v[rows16(n), :] = r[16:32]
                acc_v[rows16(n), :] = r[0:16]

            issue_to(pos[0] + 4)

        stage_lhs([_gelu(acc_v[pl.ds(8 * j, 8), :] + b1[j:j + 1]) for j in range(NF)])
        for j in range(ND):
            acc_v[pl.ds(8 * j, 8), :] = jnp.broadcast_to(b2[j:j + 1], (8, 128))
        for si in range(2):
            if si:
                issue_to(starts[-1])
            wait(g_w2 + si)
            ((kts, _, _),) = plan[si]

            @pl.loop(0, ND // 2)
            def _(n, kts=kts):
                acc_v[rows16(n), :] += _mm(staged(kts), w2_v, kts, n)

            if si == 0 and V2:
                for t in range(V2):
                    @pl.loop(0, 8)
                    def _(i, t=t):
                        w2f_v[8 * t + i] = w2_v[8 * kts0[t] + i].astype(F32)

        acc = [acc_v[pl.ds(16 * n, 16), :] for n in range(ND // 2)]
        x2 = []
        qacc = [None] * (NQ // 2)
        left = []
        for n, stage in enumerate(plan[2:]):
            wait(g_w2 + 2 + n)
            for c in range(n, ND // 2):
                kts = [k for ks, n0, n1 in stage if n0 <= c < n1 for k in ks]
                if kts:
                    _add(acc, c, _mm(staged(kts), w2_v, kts, c))
                if c == n:
                    x2 += [_rnd(x1[2 * n + i] + acc[n][8 * i:8 * i + 8]) for i in range(2)]
            for c in left:
                _add(qacc, c, _mm(xl, wq_v, 2 * n - 2, c))
            xl = _lhs_pair(x2[2 * n:])
            if n < ND // 2 - 1:
                left = range(NQ // 2 - defer, NQ // 2)
                for c in range(NQ // 2 - defer):
                    _add(qacc, c, _mm(xl, wq_v, 2 * n, c))
        m, r, _ = _stats(x2)
        m, r = jnp.concatenate([m, m], axis=0), jnp.concatenate([r, r], axis=0)
        for c in range(NQ // 2):
            put_q(c, (qacc[c] + _mm(xl, wq_v, ND - 2, c) - m * cq_v[pl.ds(16 * c, 16), :]) * r)

        def vpu_part(get_x, nt, wf_v, t0, slot):
            def spread(t, b):
                xb_v[t0 + t, b] = jnp.broadcast_to(_rnd(get_x(t))[b:b + 1], (128, 128)).T

            for b in range(B):
                spread(0, b)
            yield
            for t in range(nt):
                for n in range(ND // 2):
                    a = [[None, None] if t == 0 else [av_v[slot, 2 * n + i, pl.ds(8 * b, 8), :] for i in range(2)]
                         for b in range(B)]
                    for kc in range(16):
                        if t + 1 < nt and kc % 8 == 0:
                            spread(t + 1, 2 * n + kc // 8)
                        w = wf_v[8 * t + kc // 2, kc % 2, n]
                        for b in range(B):
                            xb = xb_v[t0 + t, b, pl.ds(8 * kc, 8), :]
                            for i in range(2):
                                _add(a[b], i, xb * w[8 * i:8 * i + 8])
                        if kc % 4 == 3:
                            yield
                    for b in range(B):
                        for i in range(2):
                            av_v[slot, 2 * n + i, pl.ds(8 * b, 8), :] = a[b][i]

        def vpu_result(gen, slot):
            for _ in gen:
                pass
            out = []
            for j in range(ND):
                r = [av_v[slot, j, pl.ds(s, 8, stride=8), :] for s in range(8)]
                out.append(((r[0] + r[1]) + (r[2] + r[3])) + ((r[4] + r[5]) + (r[6] + r[7])))
            return out

        def steps(gen, n):
            for _ in range(n):
                next(gen, None)

        acc = [None] * (ND // 2)
        vo = vpu_part(lambda t: os_v[0, pl.ds(8 * t, 8), :], VO, wof_v, 0, 0) if VO else iter(())

        def wo_block(g):
            hs = range(VO if g == 0 else 0, 8)
            if not hs:
                return
            lhs = _lhs_pair([os_v[g, pl.ds(8 * h, 8), :] for h in hs])
            for n in range(ND // 2):
                _add(acc, n, _mm(lhs, wo_v, 8 * g + hs[0], n))
                steps(vo, so)

        pend, npv = [], 0
        for g in range(G):
            for bp in range(B // 2):
                pend.append((g, bp) + scores(g, bp))
                if npv >= B // 2 + first:
                    steps(vo, sa // 2)
                if len(pend) > DEPTH:
                    pv(*pend.pop(0))
                    npv += 1
                if npv >= B // 2 + first:
                    steps(vo, sa - sa // 2)
        wo_block(0)
        wo_block(1)
        for t in pend:
            pv(*t)
            steps(vo, sa // 2)
        for g in range(2, G):
            wo_block(g)
        base = x2
        if VO:
            base = [a + b for a, b in zip(x2, vpu_result(vo, 0))]
        x3 = [_rnd(a + b) for a, b in zip(base, halves(acc))]
        m1, r1, d = _stats(x3)
        m2, r2, _ = _stats([c * r1 for c in d])
        a = r1 * r2
        cc = (m1 * r1 + m2) * r2
        HALF = ND // 2
        xl = _lhs_pair(x3)
        vk = list(kts0[:V2])
        ns = sorted(range(NF // 2), key=lambda n: not (2 * n in vk or 2 * n + 1 in vk))
        pre = {n: _mm(xl[:HALF], w1_v, 0, n) for n in ns[:NPRE]}
        h = {}
        v2 = vpu_part(lambda t: h[vk[t]], V2, w2f_v, VO, 1) if V2 else iter(())
        for ni, n in enumerate(ns):
            t = pre[n] + _mm(xl[HALF:], w1_v, HALF, n) if n in pre else _mm(xl, w1_v, 0, n)
            for i in range(2):
                j = 2 * n + i
                h[j] = _gelu(t[8 * i:8 * i + 8] * a - cc * c1_v[pl.ds(8 * j, 8), :] + b1[j:j + 1])
            if ni >= 2:
                steps(v2, s1)
        acc = [None] * (ND // 2)
        mk = [j for j in h if j not in vk]
        for j0 in range(0, len(mk), 4):
            lhs = _lhs_pair([h[j] for j in mk[j0:j0 + 4]])
            for n in range(ND // 2):
                _add(acc, n, _mm(lhs, w2_v, mk[j0:j0 + 4], n))
                steps(v2, s2)
        base = [x3[j] + b2[j:j + 1] for j in range(ND)]
        if V2:
            base = [a + b for a, b in zip(base, vpu_result(v2, 1))]
        out = [a + b for a, b in zip(base, halves(acc))]
        o_ref[...] = jnp.concatenate(out, axis=1).astype(o_ref.dtype)

    def fn(A_x, A_k_cache, A_v_cache, A_wq, A_wo, B_x, B_w1, B_b1, B_w2, B_b2):
        any_ = pl.BlockSpec(memory_space=pl.ANY)
        wq, wo, w1, w2 = (_tile_view(w) for w in (A_wq, A_wo, B_w1, B_w2))
        w1 = w1.reshape(-1, 16, 128)
        out = pl.pallas_call(
            kernel,
            out_shape=jax.ShapeDtypeStruct((B, D), A_x.dtype),
            in_specs=[any_] * 9,
            scratch_shapes=[
                pltpu.VMEM((B, D), BF),
                pltpu.VMEM((B, G, W, DH), BF),
                pltpu.VMEM((B, G, W, DH), BF),
                pltpu.VMEM(wq.shape, BF),
                pltpu.VMEM(wo.shape, BF),
                pltpu.VMEM(w1.shape, BF),
                pltpu.VMEM((NF, 128), BF),
                pltpu.VMEM(w2.shape, BF),
                pltpu.VMEM((ND, 128), BF),
                pltpu.VMEM((B, G, W // 128, DH, 128), BF),
                pltpu.VMEM((G, HQ // G * B, DH), F32),
                pltpu.VMEM((G, HQ // G * B, DH), F32),
                pltpu.VMEM((NQ * 8, 128), F32),
                pltpu.VMEM((NF * 8, 128), F32),
                pltpu.VMEM((NQ, 2, 32, 128), BF),
                pltpu.VMEM((NF * 8, 128), F32),
                pltpu.VMEM((8 * max(VO, 1), 2, ND // 2, 16, 128), F32),
                pltpu.VMEM((8 * max(V2, 1), 2, ND // 2, 16, 128), F32),
                pltpu.VMEM((max(VO + V2, 1), B, 128, 128), F32),
                pltpu.VMEM((2, ND, 64, 128), F32),
                pltpu.SemaphoreType.DMA((8 + len(plan),)),
            ],
            compiler_params=pltpu.CompilerParams(
                vmem_limit_bytes=100 * 1024 * 1024, disable_semaphore_checks=True, disable_bounds_checks=True),
        )(A_x.reshape(B, D), A_k_cache, A_v_cache, wq, wo, w1, B_b1.reshape(NF, 128), w2, B_b2.reshape(ND, 128))
        return out.reshape(A_x.shape)

    return fn


@jax.jit
def pallas_interleave_layers__sliding_block_cached__mixer_channel_mlp__decode_kernel(
    A_x, A_k_cache, A_v_cache, A_wq, A_wo, B_x, B_w1, B_b1, B_w2, B_b2
):
    return make(STAIR, 24)(A_x, A_k_cache, A_v_cache, A_wq, A_wo, B_x, B_w1, B_b1, B_w2, B_b2)
```

```python
import jax
import jax.numpy as jnp
import numpy as np
from jax import lax
import jax.experimental.pallas as pl
import jax.experimental.pallas.tpu as pltpu

BF = jnp.bfloat16
F32 = jnp.float32
EPS = 1e-5
HQ, DH = 32, 128
S = 8


def _tile_view(w):
    K, N = w.shape
    w = w.reshape(K // 16, 2, 8, N // 256, 2, 128).transpose(0, 1, 3, 4, 2, 5)
    return w.reshape(K // 16, 2, N // 256, 16, 128)


def _lhs_pair(cols):
    even = (lax.broadcasted_iota(jnp.int32, (8, 128), 1) & 8) == 0
    out = []
    for x in cols:
        xe, xo = jnp.where(even, x, 0.0), jnp.where(even, 0.0, x)
        out.append((jnp.concatenate([xe, pltpu.roll(xe, 8, 1)], axis=0).astype(BF),
                    jnp.concatenate([pltpu.roll(xo, 120, 1), xo], axis=0).astype(BF)))
    return out


def _dot(lhs, rhs):
    return jnp.dot(jnp.concatenate(lhs, axis=1), jnp.concatenate(rhs, axis=0), preferred_element_type=F32)


def _mm(lhs, tile, kts, n):
    a, b = (_dot([t[p] for t in lhs], [tile(k, p, n) for k in kts]) for p in range(2))
    return a + b


def _rowmean(cols):
    t = cols[0]
    for c in cols[1:]:
        t = t + c
    return jnp.sum(t, axis=1, keepdims=True) * (1.0 / (128 * len(cols)))


def _stats(cols):
    m = _rowmean(cols)
    d = [c - m for c in cols]
    return m, lax.rsqrt(_rowmean([c * c for c in d]) + EPS), d


def _ln(cols):
    _, r, d = _stats(cols)
    return [c * r for c in d]


def _gelu(x):
    c = np.float32(np.sqrt(2.0 / np.pi))
    return 0.5 * x * (1.0 + jnp.tanh(c * (x + 0.044715 * (x * x * x))))


def _rnd(x):
    return x.astype(BF).astype(F32)


def _add(acc, n, r):
    acc[n] = r if acc[n] is None else acc[n] + r


def _w2_plan(d=6, e=3, f=3, g=2):
    order = [(i * 11) % 28 for i in range(28)]

    def take(n):
        return tuple(sorted(order.pop() for _ in range(n)))

    d, e, f, g, r = take(d), take(e), take(f), take(g), take(8)
    rest = take(len(order))
    return [[(r, 0, 8)], [(rest, 0, 8)], [(d + e, 0, 6)],
            [(f, 0, 4), (g, 0, 2)], [(g, 2, 8)], [(f, 4, 8)], [(e, 6, 8), (d, 6, 7)], [(d, 7, 8)]]


def make(plan=None, shift=24, lag=14, depth=2, defer=(8, 8, 8, 16), npre=4, bc=False, nobc=False):
    B, D, G, W, F = 8, 1024, 4, 1024, 3584
    ND, NQ, NF, REP = D // 128, HQ * DH // 128, F // 128, HQ // G
    plan = plan or _w2_plan()
    pieces = [p for stage in plan for p in stage]
    thin = plan[-1][0][0]

    def _ld(ref, idx):
        if bc:
            return pltpu.bitcast(ref.bitcast(jnp.int32)[idx].reshape(-1, 128), BF)
        return ref[idx].reshape(-1, 128)

    def kernel(x_h, k_h, v_h, wq_h, wo_h, w1_h, b1_h, w2_h, w2flat_h, b2_h, o_ref,
               x_v, k_v, v_v, wq_v, wo_v, w1_v, b1_v, b2_v, kt_v, qs_v, os_v, cq_v, c1_v,
               lhs_v, nat_v, acc_v, sems, *w2_v):
        Sk = k_h.shape[2]

        rounds, filled = [], []

        def streamed(n, src, dst, idx, src_idx=None):
            sem = sems.at[len(filled)]

            def issue(t):
                for s in range(S):
                    pltpu.make_async_copy(
                        src.at[(src_idx or idx)(s, t)], dst.at[idx(s, t)], sem).start(priority=s % 2)

            rounds.append((n, issue))
            filled.append(dst)
            return len(filled) - 1

        def kv_idx(off):
            return lambda s, t: (s, t >> 3, pl.ds(pl.multiple_of(off + (t & 7) * 128, 128), 128))

        g_wq = streamed(32, wq_h, wq_v, lambda s, t: (s * 8 + (t >> 2), (t >> 1) & 1, pl.ds((t & 1) * 8, 8)))
        g_k = streamed(32, k_h, k_v, kv_idx(0), kv_idx(Sk - W))
        g_v = streamed(32, v_h, v_v, kv_idx(0), kv_idx(Sk - W))
        g_wo = streamed(32, wo_h, wo_v, lambda s, t: (s * 32 + t,))
        g_w1 = streamed(28, w1_h, w1_v, lambda s, t: (pl.ds((s * 28 + t) * 8, 8),))
        copies = []
        for (kts, c0, c1), dst in zip(pieces, w2_v):
            if c1 - c0 == 1:
                part = [(w2flat_h.at[pl.ds(128 * k, 128), pl.ds(128 * c0, 128)], dst.at[j])
                        for j, k in enumerate(kts)]
            else:
                per = 8 // (c1 - c0)
                part = [(w2_h.at[pl.ds(8 * k + i, per), :, pl.ds(c0 // 2, (c1 - c0) // 2)],
                         dst.at[pl.ds(8 * j + i, per)])
                        for i in range(0, 8, per) for j, k in enumerate(kts)]
            copies += [(a, b, sems.at[len(filled)]) for a, b in part]
            filled.append(dst)
        n0 = 8 * len(pieces[0][0])
        head = copies[n0:len(copies) - shift]
        q0, q1 = head[0::2], head[1::2] + copies[len(copies) - shift:]
        lead = len(q1) - len(q0)
        order = [(c, i % 2) for i, c in enumerate(copies[:n0])] + [(c, 1) for c in q1[:lead]]
        order += [x for a, b in zip(q0, q1[lead:]) for x in ((a, 0), (b, 1))]
        for i in range(0, len(order), S):
            def issue(t, part=order[i:i + S]):
                for c, queue in part:
                    pltpu.make_async_copy(*c).start(priority=queue)

            rounds.append((1, issue))
        starts = [int(v) for v in np.cumsum([0] + [r[0] for r in rounds])]
        pos = [0]

        def issue_to(hi, body=None, per=1):
            hi, done = min(hi, starts[-1]), 0
            for (n, issue), lo, end in zip(rounds, starts, starts[1:]):
                a, b = max(pos[0], lo), min(hi, end)
                if a >= b:
                    continue
                assert (b - a) % per == 0

                def step(t, issue=issue, t0=a - lo, done=done):
                    for u in range(per):
                        issue(t0 + t * per + u)
                    if body is not None:
                        body(done + t)

                if n == 1:
                    step(0)
                else:
                    pl.loop(0, (b - a) // per)(step)
                done += (b - a) // per
            pos[0] = max(pos[0], hi)

        def overlapped(n, per=1):
            return lambda body: issue_to(pos[0] + n * per, body, per)

        def wait(i):
            pltpu.make_async_copy(filled[i], filled[i], sems.at[i]).wait()

        def landed(i):
            issue_to(starts[i + 1] + lag)
            wait(i)

        def wait_stage(si):
            assert pos[0] >= (starts[-1] if si else starts[g_w1 + 1] + n0 // S)
            for p in plan[si]:
                wait(g_w1 + 1 + pieces.index(p))

        def tiles(ref):
            return lambda k, p, n: _ld(ref, (pl.ds(8 * k, 8), p, n))

        def w1_tile(k, p, n):
            return jnp.concatenate(
                [_ld(w1_v, ((8 * k + i) * NF + p * (NF // 2) + n,)) for i in range(8)], axis=0)

        def w2_piece(k, c):
            return next((ref, kts.index(k), c0) for (kts, c0, c1), ref in zip(pieces, w2_v)
                        if k in kts and c0 <= c < c1)

        def w2_tile(k, p, n):
            ref, j, c0 = w2_piece(k, 2 * n)
            return _ld(ref, (pl.ds(8 * j, 8), p, n - c0 // 2))

        def thin_mm(lhs, c):
            return _dot(lhs, [_ld(w2_piece(k, c)[0], (j,)) for j, k in enumerate(thin)])[0:8]

        def stage_lhs(cols, k0=0, ones=False):
            lane = lax.broadcasted_iota(jnp.int32, (16, 128), 1)
            row = lax.broadcasted_iota(jnp.int32, (16, 128), 0)
            one = jnp.where((lane & 8) == (row & 8), 1.0, 0.0).astype(BF)
            for k, t in enumerate(_lhs_pair(cols)):
                for p in range(2):
                    lhs_v[k0 + k, p, pl.ds(0, 16), :] = t[p]
                    if ones:
                        lhs_v[k0 + k, p, pl.ds(16, 16), :] = one

        def staged(kts, m=16):
            return [tuple(lhs_v[k, p, pl.ds(0, m), :] for p in range(2)) for k in kts]

        def rows16(n):
            return pl.ds(pl.multiple_of(16 * n, 16), 16)

        def halves(acc):
            return [a[8 * i:8 * i + 8] for a in acc for i in range(2)]

        def put_q(n, q):
            qs_v[n >> 2, rows16(n & 3), :] = _rnd(q) * np.float32(DH ** -0.5)

        def scores(g, bp):
            q = jnp.concatenate(
                [qs_v[g, pl.ds(2 * bp + i, REP, stride=B), :] for i in range(2)], axis=0).astype(BF)
            s = []
            for i in range(2):
                kt = jnp.concatenate([_ld(kt_v, (2 * bp + i, g, j)) for j in range(W // 128)], axis=1)
                s.append(jnp.dot(q, kt, preferred_element_type=F32)[8 * i:8 * i + 8])
            s = jnp.concatenate(s, axis=0)
            e = jnp.exp(s - jnp.max(s, axis=1, keepdims=True))
            return e.astype(BF), 1.0 / jnp.sum(e, axis=1, keepdims=True)

        def pv(g, bp, p, linv):
            for i in range(2):
                o = jnp.dot(p, _ld(v_v, (2 * bp + i, g)), preferred_element_type=F32)
                os_v[g, pl.ds(2 * bp + i, REP, stride=B), :] = o[8 * i:8 * i + 8] * linv[8 * i:8 * i + 8]

        def heads(g):
            return [os_v[g, pl.ds(B * h, B), :] for h in range(REP)]

        small = [pltpu.make_async_copy(h, v, sems.at[len(filled) + i])
                 for i, (h, v) in enumerate(((x_h, x_v), (b1_h, b1_v), (b2_h, b2_v)))]
        issue_to(1)
        for c in small:
            c.start()
        landed(g_wq)
        for c in small:
            c.wait()
        x0 = x_v[...].astype(F32)
        x0 = [x0[:, 128 * j:128 * j + 128] for j in range(ND)]
        stage_lhs(_ln(x0), ones=True)
        acc_v[pl.ds(0, 8 * ND), :] = jnp.concatenate(x0, axis=0)

        @overlapped(NQ // 2)
        def _(n):
            r = _mm(staged(range(ND), 32), tiles(wq_v), range(ND), n)
            cq_v[rows16(n), :] = r[16:32]
            put_q(n, r[0:16])

        landed(g_k)

        @overlapped(B * G)
        def _(i):
            b, g = i >> 2, i & 3
            for j in range(W // 128):
                kt_v[b, g, j] = k_v[b, g, pl.ds(128 * j, 128), :].T

        landed(g_v)

        @overlapped(G * B // 2, 2)
        def _(i):
            g, bp = i >> 2, i & 3
            pv(g, bp, *scores(g, bp))

        @pl.loop(0, G)
        def _(g):
            stage_lhs(heads(g), REP * g)

        landed(g_wo)

        @overlapped(G * ND // 2)
        def _(i):
            g, n = i >> 2, i & 3
            kts = [REP * g + h for h in range(REP)]
            acc_v[rows16(n), :] += _mm(staged(kts), tiles(wo_v), kts, n)

        x1 = [_rnd(acc_v[pl.ds(8 * j, 8), :]) for j in range(ND)]
        stage_lhs(_ln(_ln(x1)), ones=True)
        landed(g_w1)
        b1 = b1_v[...].astype(F32)
        b2 = b2_v[...].astype(F32)
        for i in range(2):
            @pl.loop(i * NF // 4, (i + 1) * NF // 4)
            def _(n):
                r = _mm(staged(range(ND), 32), w1_tile, range(ND), n)
                c1_v[rows16(n), :] = r[16:32]
                acc_v[rows16(n), :] = r[0:16]

            issue_to(pos[0] + 4)

        h = [_gelu(acc_v[pl.ds(8 * j, 8), :] + b1[j:j + 1]) for j in range(NF)]
        stage_lhs(h)
        for j, k in enumerate(thin):
            nat_v[j] = jnp.concatenate([h[k], h[k]], axis=0).astype(BF)
        for j in range(ND):
            acc_v[pl.ds(8 * j, 8), :] = jnp.broadcast_to(b2[j:j + 1], (8, 128))
        for si in range(3):
            if si == 1:
                issue_to(starts[-1])
            wait_stage(si)
            ((kts, _, c1),) = plan[si]

            @pl.loop(0, c1 // 2)
            def _(n, kts=kts, ref=w2_v[si]):
                acc_v[rows16(n), :] += _mm(staged(kts), tiles(ref), range(len(kts)), n)

        acc = [acc_v[pl.ds(8 * j, 8), :] for j in range(ND)]
        x2, left, qacc = [], [], [None] * (NQ // 2)
        for si, upto in enumerate((2, 4, 6, 7, 8)):
            wait_stage(3 + si)
            for n in range(ND // 2):
                kts = [k for ks, c0, c1 in plan[3 + si] if c0 <= 2 * n and 2 * n + 1 < c1 for k in ks]
                if kts:
                    r = _mm(staged(kts), w2_tile, kts, n)
                    _add(acc, 2 * n, r[0:8])
                    _add(acc, 2 * n + 1, r[8:16])
            if upto > 6:
                _add(acc, upto - 1, thin_mm([nat_v[j] for j in range(len(thin))], upto - 1))
            kts = range(len(x2), upto)
            x2 += [_rnd(x1[j] + acc[j]) for j in kts]
            left += [(_lhs_pair(x2[kts[0]:]), kts, n) for n in range(NQ // 2)]
            while upto < ND and len(left) > defer[si]:
                xl, ks, n = left.pop(0)
                _add(qacc, n, _mm(xl, tiles(wq_v), ks, n))
        m, r, _ = _stats(x2)
        m, r = jnp.concatenate([m, m], axis=0), jnp.concatenate([r, r], axis=0)
        for xl, ks, n in left:
            _add(qacc, n, _mm(xl, tiles(wq_v), ks, n))
            if ks[-1] == ND - 1:
                put_q(n, (qacc[n] - m * cq_v[pl.ds(16 * n, 16), :]) * r)

        acc = [None] * (ND // 2)

        def wo_block(g):
            lhs = _lhs_pair(heads(g))
            for n in range(ND // 2):
                _add(acc, n, _mm(lhs, tiles(wo_v), range(REP * g, REP * (g + 1)), n))

        pend = []
        for g in range(G):
            for bp in range(B // 2):
                pend.append((g, bp) + scores(g, bp))
                if len(pend) > depth:
                    pv(*pend.pop(0))
        wo_block(0)
        for t in pend:
            pv(*t)
        for g in range(1, G):
            wo_block(g)
        x3 = [_rnd(a + b) for a, b in zip(x2, halves(acc))]

        m1, r1, d = _stats(x3)
        m2, r2, _ = _stats([c * r1 for c in d])
        scale, offset = r1 * r2, (m1 * r1 + m2) * r2
        xl = _lhs_pair(x3)
        lo, hi = range(ND // 2), range(ND // 2, ND)
        pre = [_mm(xl[:ND // 2], w1_tile, lo, n) for n in range(npre)]
        h = []
        for n in range(NF // 2):
            t = pre[n] + _mm(xl[ND // 2:], w1_tile, hi, n) if n < npre else _mm(xl, w1_tile, range(ND), n)
            for j in (2 * n, 2 * n + 1):
                h.append(_gelu(t[8 * (j % 2):8 * (j % 2) + 8] * scale
                               - offset * c1_v[pl.ds(8 * j, 8), :] + b1[j:j + 1]))
        acc = [None] * (ND // 2)
        for k0 in range(0, NF, 4):
            lhs = _lhs_pair(h[k0:k0 + 4])
            for n in range(ND // 2):
                kts = [k for k in range(k0, k0 + 4) if n < 3 or k not in thin]
                _add(acc, n, _mm([lhs[k - k0] for k in kts], w2_tile, kts, n))
            if k0 == 8:
                nat = [jnp.concatenate([h[k], h[k]], axis=0).astype(BF) for k in thin]
                _add(acc, 3, jnp.concatenate([thin_mm(nat, 6), thin_mm(nat, 7)], axis=0))
        out = [(x3[j] + b2[j:j + 1]) + t for j, t in enumerate(halves(acc))]
        o_ref[...] = jnp.concatenate(out, axis=1).astype(o_ref.dtype)

    def fn(A_x, A_k_cache, A_v_cache, A_wq, A_wo, B_x, B_w1, B_b1, B_w2, B_b2):
        Sk = A_k_cache.shape[2]
        assert A_x.shape == (B, 1, D) and A_k_cache.shape == (B, G, Sk, DH) and B_w1.shape == (D, F)
        assert min(4096, max(256, Sk // 4)) == W and Sk % 128 == 0
        wq, wo, w1, w2 = (_tile_view(w) for w in (A_wq, A_wo, B_w1, B_w2))
        w1 = w1.reshape(-1, 16, 128)
        out = pl.pallas_call(
            kernel,
            out_shape=jax.ShapeDtypeStruct((B, D), A_x.dtype),
            in_specs=[pl.BlockSpec(memory_space=pl.ANY)] * 10,
            scratch_shapes=[
                pltpu.VMEM((B, D), BF),
                pltpu.VMEM((B, G, W, DH), BF),
                pltpu.VMEM((B, G, W, DH), BF),
                pltpu.VMEM(wq.shape, BF),
                pltpu.VMEM(wo.shape, BF),
                pltpu.VMEM(w1.shape, BF),
                pltpu.VMEM((NF, 128), BF),
                pltpu.VMEM((ND, 128), BF),
                pltpu.VMEM((B, G, W // 128, DH, 128), BF),
                pltpu.VMEM((G, (REP + 1) * B, DH), F32),
                pltpu.VMEM((G, (REP + 1) * B, DH), F32),
                pltpu.VMEM((NQ * 8, 128), F32),
                pltpu.VMEM((NF * 8, 128), F32),
                pltpu.VMEM((NQ, 2, 32, 128), BF),
                pltpu.VMEM((len(thin), 16, 128), BF),
                pltpu.VMEM((NF * 8, 128), F32),
                pltpu.SemaphoreType.DMA((8 + len(pieces),)),
            ] + [
                pltpu.VMEM((len(kts), 128, 128) if c1 - c0 == 1
                           else (8 * len(kts), 2, (c1 - c0) // 2, 16, 128), BF)
                for kts, c0, c1 in pieces
            ],
            compiler_params=pltpu.CompilerParams(
                vmem_limit_bytes=100 * 1024 * 1024, disable_semaphore_checks=True, disable_bounds_checks=nobc),
        )(A_x.reshape(B, D), A_k_cache, A_v_cache, wq, wo, w1, B_b1.reshape(NF, 128),
          w2, B_w2, B_b2.reshape(ND, 128))
        return out.reshape(A_x.shape)

    return fn


@jax.jit
def pallas_interleave_layers__sliding_block_cached__mixer_channel_mlp__decode_kernel(
    A_x, A_k_cache, A_v_cache, A_wq, A_wo, B_x, B_w1, B_b1, B_w2, B_b2
):
    return make()(A_x, A_k_cache, A_v_cache, A_wq, A_wo, B_x, B_w1, B_b1, B_w2, B_b2)
```

```python
import jax
import jax.numpy as jnp
import numpy as np
from jax import lax
import jax.experimental.pallas as pl
import jax.experimental.pallas.tpu as pltpu

BF = jnp.bfloat16
F32 = jnp.float32
EPS = 1e-5
B, D, F = 8, 1024, 3584
HQ, G, DH, W = 32, 4, 128, 1024
ND, NQ, NF, REP = D // 128, HQ * DH // 128, F // 128, HQ // G
S = 8


def _tile_view(w):
    K, N = w.shape
    w = w.reshape(K // 16, 2, 8, N // 256, 2, 128).transpose(0, 1, 3, 4, 2, 5)
    return w.reshape(K // 16, 2, N // 256, 16, 128)


def _lhs_pair(cols):
    even = (lax.broadcasted_iota(jnp.int32, (8, 128), 1) & 8) == 0
    out = []
    for x in cols:
        xe, xo = jnp.where(even, x, 0.0), jnp.where(even, 0.0, x)
        out.append((jnp.concatenate([xe, pltpu.roll(xe, 8, 1)], axis=0).astype(BF),
                    jnp.concatenate([pltpu.roll(xo, 120, 1), xo], axis=0).astype(BF)))
    return out


def _dot(lhs, rhs):
    return jnp.dot(jnp.concatenate(lhs, axis=1), jnp.concatenate(rhs, axis=0), preferred_element_type=F32)


def _mm(lhs, tile, kts, n):
    a, b = (_dot([t[p] for t in lhs], [tile(k, p, n) for k in kts]) for p in range(2))
    return a + b


def _rowmean(cols):
    t = cols[0]
    for c in cols[1:]:
        t = t + c
    return jnp.broadcast_to(jnp.sum(t, axis=1, keepdims=True), t.shape) * (1.0 / (128 * len(cols)))


def _stats(cols):
    m = _rowmean(cols)
    d = [c - m for c in cols]
    return m, lax.rsqrt(_rowmean([c * c for c in d]) + EPS), d


def _ln(cols):
    _, r, d = _stats(cols)
    return [c * r for c in d]


def _gelu(x):
    c = np.float32(np.sqrt(2.0 / np.pi))
    return 0.5 * x * (1.0 + jnp.tanh(c * (x + 0.044715 * (x * x * x))))


def _rnd(x):
    return x.astype(BF).astype(F32)


def _add(acc, n, r):
    acc[n] = r if acc[n] is None else acc[n] + r


def _w2_plan(d=6, e=3, f=3, g=2):
    order = [(i * 11) % 28 for i in range(28)]

    def take(n):
        return tuple(sorted(order.pop() for _ in range(n)))

    d, e, f, g, r = take(d), take(e), take(f), take(g), take(8)
    rest = take(len(order))
    return [[(r, 0, 8)], [(rest, 0, 8)], [(d + e, 0, 6)],
            [(f, 0, 4), (g, 0, 2)], [(g, 2, 8)], [(f, 4, 8)], [(e, 6, 8), (d, 6, 7)], [(d, 7, 8)]]


PLAN = _w2_plan()
PIECES = [p for stage in PLAN for p in stage]
THIN = PLAN[-1][0][0]
LAG = 14
SHIFT = 24
DEFER = (8, 8, 8, 16)
DEPTH = 2
NPRE = 4


def _ld(ref, idx):
    return ref[idx].reshape(-1, 128)


def _kernel(x_h, k_h, v_h, wq_h, wo_h, w1_h, b1_h, w2_h, w2flat_h, b2_h, o_ref,
            x_v, k_v, v_v, wq_v, wo_v, w1_v, b1_v, b2_v, kt_v, qs_v, os_v, cq_v, c1_v,
            lhs_v, nat_v, acc_v, sems, *w2_v):
    Sk = k_h.shape[2]

    rounds, filled = [], []

    def streamed(n, src, dst, idx, src_idx=None):
        sem = sems.at[len(filled)]

        def issue(t):
            for s in range(S):
                pltpu.make_async_copy(
                    src.at[(src_idx or idx)(s, t)], dst.at[idx(s, t)], sem).start(priority=s % 2)

        rounds.append((n, issue))
        filled.append(dst)
        return len(filled) - 1

    def kv_idx(off):
        return lambda s, t: (s, t >> 3, pl.ds(pl.multiple_of(off + (t & 7) * 128, 128), 128))

    g_wq = streamed(32, wq_h, wq_v, lambda s, t: (s * 8 + (t >> 2), (t >> 1) & 1, pl.ds((t & 1) * 8, 8)))
    g_k = streamed(32, k_h, k_v, kv_idx(0), kv_idx(Sk - W))
    g_v = streamed(32, v_h, v_v, kv_idx(0), kv_idx(Sk - W))
    g_wo = streamed(32, wo_h, wo_v, lambda s, t: (s * 32 + t,))
    g_w1 = streamed(28, w1_h, w1_v, lambda s, t: (pl.ds((s * 28 + t) * 8, 8),))
    copies = []
    for (kts, c0, c1), dst in zip(PIECES, w2_v):
        if c1 - c0 == 1:
            part = [(w2flat_h.at[pl.ds(128 * k, 128), pl.ds(128 * c0, 128)], dst.at[j])
                    for j, k in enumerate(kts)]
        else:
            per = 8 // (c1 - c0)
            part = [(w2_h.at[pl.ds(8 * k + i, per), :, pl.ds(c0 // 2, (c1 - c0) // 2)],
                     dst.at[pl.ds(8 * j + i, per)])
                    for i in range(0, 8, per) for j, k in enumerate(kts)]
        copies += [(a, b, sems.at[len(filled)]) for a, b in part]
        filled.append(dst)
    n0 = 8 * len(PIECES[0][0])
    head = copies[n0:len(copies) - SHIFT]
    q0, q1 = head[0::2], head[1::2] + copies[len(copies) - SHIFT:]
    lead = len(q1) - len(q0)
    order = [(c, i % 2) for i, c in enumerate(copies[:n0])] + [(c, 1) for c in q1[:lead]]
    order += [x for a, b in zip(q0, q1[lead:]) for x in ((a, 0), (b, 1))]
    for i in range(0, len(order), S):
        def issue(t, part=order[i:i + S]):
            for c, queue in part:
                pltpu.make_async_copy(*c).start(priority=queue)

        rounds.append((1, issue))
    starts = [int(v) for v in np.cumsum([0] + [r[0] for r in rounds])]
    pos = [0]

    def issue_to(hi, body=None, per=1):
        hi, done = min(hi, starts[-1]), 0
        for (n, issue), lo, end in zip(rounds, starts, starts[1:]):
            a, b = max(pos[0], lo), min(hi, end)
            if a >= b:
                continue
            assert (b - a) % per == 0

            def step(t, issue=issue, t0=a - lo, done=done):
                for u in range(per):
                    issue(t0 + t * per + u)
                if body is not None:
                    body(done + t)

            if n == 1:
                step(0)
            else:
                pl.loop(0, (b - a) // per)(step)
            done += (b - a) // per
        pos[0] = max(pos[0], hi)

    def overlapped(n, per=1):
        return lambda body: issue_to(pos[0] + n * per, body, per)

    def wait(i):
        pltpu.make_async_copy(filled[i], filled[i], sems.at[i]).wait()

    def landed(i):
        issue_to(starts[i + 1] + LAG)
        wait(i)

    def wait_stage(si):
        assert pos[0] >= (starts[-1] if si else starts[g_w1 + 1] + n0 // S)
        for p in PLAN[si]:
            wait(g_w1 + 1 + PIECES.index(p))

    def tiles(ref):
        return lambda k, p, n: _ld(ref, (pl.ds(8 * k, 8), p, n))

    def w1_tile(k, p, n):
        return jnp.concatenate(
            [_ld(w1_v, ((8 * k + i) * NF + p * (NF // 2) + n,)) for i in range(8)], axis=0)

    def w2_piece(k, c):
        return next((ref, kts.index(k), c0) for (kts, c0, c1), ref in zip(PIECES, w2_v)
                    if k in kts and c0 <= c < c1)

    def w2_tile(k, p, n):
        ref, j, c0 = w2_piece(k, 2 * n)
        return _ld(ref, (pl.ds(8 * j, 8), p, n - c0 // 2))

    def thin_mm(lhs, c):
        return _dot(lhs, [_ld(w2_piece(k, c)[0], (j,)) for j, k in enumerate(THIN)])[0:8]

    def stage_lhs(cols, k0=0, ones=False):
        lane = lax.broadcasted_iota(jnp.int32, (16, 128), 1)
        row = lax.broadcasted_iota(jnp.int32, (16, 128), 0)
        one = jnp.where((lane & 8) == (row & 8), 1.0, 0.0).astype(BF)
        for k, t in enumerate(_lhs_pair(cols)):
            for p in range(2):
                lhs_v[k0 + k, p, pl.ds(0, 16), :] = t[p]
                if ones:
                    lhs_v[k0 + k, p, pl.ds(16, 16), :] = one

    def staged(kts, m=16):
        return [tuple(lhs_v[k, p, pl.ds(0, m), :] for p in range(2)) for k in kts]

    def rows16(n):
        return pl.ds(pl.multiple_of(16 * n, 16), 16)

    def halves(acc):
        return [a[8 * i:8 * i + 8] for a in acc for i in range(2)]

    def put_q(n, q):
        qs_v[n >> 2, rows16(n & 3), :] = _rnd(q) * np.float32(DH ** -0.5)

    def scores(g, bp):
        q = jnp.concatenate(
            [qs_v[g, pl.ds(2 * bp + i, REP, stride=B), :] for i in range(2)], axis=0).astype(BF)
        s = []
        for i in range(2):
            kt = jnp.concatenate([_ld(kt_v, (2 * bp + i, g, j)) for j in range(W // 128)], axis=1)
            s.append(jnp.dot(q, kt, preferred_element_type=F32)[8 * i:8 * i + 8])
        s = jnp.concatenate(s, axis=0)
        e = jnp.exp(s - jnp.max(s, axis=1, keepdims=True))
        return e.astype(BF), 1.0 / jnp.broadcast_to(jnp.sum(e, axis=1, keepdims=True), (16, DH))

    def pv(g, bp, p, linv):
        for i in range(2):
            o = jnp.dot(p, _ld(v_v, (2 * bp + i, g)), preferred_element_type=F32)
            os_v[g, pl.ds(2 * bp + i, REP, stride=B), :] = o[8 * i:8 * i + 8] * linv[8 * i:8 * i + 8]

    def heads(g):
        return [os_v[g, pl.ds(B * h, B), :] for h in range(REP)]

    small = [pltpu.make_async_copy(h, v, sems.at[len(filled) + i])
             for i, (h, v) in enumerate(((x_h, x_v), (b1_h, b1_v), (b2_h, b2_v)))]
    issue_to(1)
    for c in small:
        c.start()
    landed(g_wq)
    for c in small:
        c.wait()
    x0 = x_v[...].astype(F32)
    x0 = [x0[:, 128 * j:128 * j + 128] for j in range(ND)]
    stage_lhs(_ln(x0), ones=True)
    acc_v[pl.ds(0, 8 * ND), :] = jnp.concatenate(x0, axis=0)

    @overlapped(NQ // 2)
    def _(n):
        r = _mm(staged(range(ND), 32), tiles(wq_v), range(ND), n)
        cq_v[rows16(n), :] = r[16:32]
        put_q(n, r[0:16])

    landed(g_k)

    @overlapped(B * G)
    def _(i):
        b, g = i >> 2, i & 3
        for j in range(W // 128):
            kt_v[b, g, j] = k_v[b, g, pl.ds(128 * j, 128), :].T

    landed(g_v)

    @overlapped(G * B // 2, 2)
    def _(i):
        g, bp = i >> 2, i & 3
        pv(g, bp, *scores(g, bp))

    @pl.loop(0, G)
    def _(g):
        stage_lhs(heads(g), REP * g)

    landed(g_wo)

    @overlapped(G * ND // 2)
    def _(i):
        g, n = i >> 2, i & 3
        kts = [REP * g + h for h in range(REP)]
        acc_v[rows16(n), :] += _mm(staged(kts), tiles(wo_v), kts, n)

    x1 = [_rnd(acc_v[pl.ds(8 * j, 8), :]) for j in range(ND)]
    stage_lhs(_ln(_ln(x1)), ones=True)
    landed(g_w1)
    b1 = b1_v[...].astype(F32)
    b2 = b2_v[...].astype(F32)
    for i in range(2):
        @pl.loop(i * NF // 4, (i + 1) * NF // 4)
        def _(n):
            r = _mm(staged(range(ND), 32), w1_tile, range(ND), n)
            c1_v[rows16(n), :] = r[16:32]
            acc_v[rows16(n), :] = r[0:16]

        issue_to(pos[0] + 4)

    h = [_gelu(acc_v[pl.ds(8 * j, 8), :] + b1[j:j + 1]) for j in range(NF)]
    stage_lhs(h)
    for j, k in enumerate(THIN):
        nat_v[j] = jnp.concatenate([h[k], h[k]], axis=0).astype(BF)
    for j in range(ND):
        acc_v[pl.ds(8 * j, 8), :] = jnp.broadcast_to(b2[j:j + 1], (8, 128))
    for si in range(3):
        if si == 1:
            issue_to(starts[-1])
        wait_stage(si)
        ((kts, _, c1),) = PLAN[si]

        @pl.loop(0, c1 // 2)
        def _(n, kts=kts, ref=w2_v[si]):
            acc_v[rows16(n), :] += _mm(staged(kts), tiles(ref), range(len(kts)), n)

    acc = [acc_v[pl.ds(8 * j, 8), :] for j in range(ND)]
    x2, left, qacc = [], [], [None] * (NQ // 2)
    for si, upto in enumerate((2, 4, 6, 7, 8)):
        wait_stage(3 + si)
        for n in range(ND // 2):
            kts = [k for ks, c0, c1 in PLAN[3 + si] if c0 <= 2 * n and 2 * n + 1 < c1 for k in ks]
            if kts:
                r = _mm(staged(kts), w2_tile, kts, n)
                _add(acc, 2 * n, r[0:8])
                _add(acc, 2 * n + 1, r[8:16])
        if upto > 6:
            _add(acc, upto - 1, thin_mm([nat_v[j] for j in range(len(THIN))], upto - 1))
        kts = range(len(x2), upto)
        x2 += [_rnd(x1[j] + acc[j]) for j in kts]
        left += [(_lhs_pair(x2[kts[0]:]), kts, n) for n in range(NQ // 2)]
        while upto < ND and len(left) > DEFER[si]:
            xl, ks, n = left.pop(0)
            _add(qacc, n, _mm(xl, tiles(wq_v), ks, n))
    m, r, _ = _stats(x2)
    m, r = jnp.concatenate([m, m], axis=0), jnp.concatenate([r, r], axis=0)
    for xl, ks, n in left:
        _add(qacc, n, _mm(xl, tiles(wq_v), ks, n))
        if ks[-1] == ND - 1:
            put_q(n, (qacc[n] - m * cq_v[pl.ds(16 * n, 16), :]) * r)

    acc = [None] * (ND // 2)

    def wo_block(g):
        lhs = _lhs_pair(heads(g))
        for n in range(ND // 2):
            _add(acc, n, _mm(lhs, tiles(wo_v), range(REP * g, REP * (g + 1)), n))

    pend = []
    for g in range(G):
        for bp in range(B // 2):
            pend.append((g, bp) + scores(g, bp))
            if len(pend) > DEPTH:
                pv(*pend.pop(0))
    wo_block(0)
    for t in pend:
        pv(*t)
    for g in range(1, G):
        wo_block(g)
    x3 = [_rnd(a + b) for a, b in zip(x2, halves(acc))]

    m1, r1, d = _stats(x3)
    m2, r2, _ = _stats([c * r1 for c in d])
    scale, offset = r1 * r2, (m1 * r1 + m2) * r2
    xl = _lhs_pair(x3)
    lo, hi = range(ND // 2), range(ND // 2, ND)
    pre = [_mm(xl[:ND // 2], w1_tile, lo, n) for n in range(NPRE)]
    h = []
    for n in range(NF // 2):
        t = pre[n] + _mm(xl[ND // 2:], w1_tile, hi, n) if n < NPRE else _mm(xl, w1_tile, range(ND), n)
        for j in (2 * n, 2 * n + 1):
            h.append(_gelu(t[8 * (j % 2):8 * (j % 2) + 8] * scale
                           - offset * c1_v[pl.ds(8 * j, 8), :] + b1[j:j + 1]))
    acc = [None] * (ND // 2)
    for k0 in range(0, NF, 4):
        lhs = _lhs_pair(h[k0:k0 + 4])
        for n in range(ND // 2):
            kts = [k for k in range(k0, k0 + 4) if n < 3 or k not in THIN]
            _add(acc, n, _mm([lhs[k - k0] for k in kts], w2_tile, kts, n))
        if k0 == 8:
            nat = [jnp.concatenate([h[k], h[k]], axis=0).astype(BF) for k in THIN]
            _add(acc, 3, jnp.concatenate([thin_mm(nat, 6), thin_mm(nat, 7)], axis=0))
    out = [(x3[j] + b2[j:j + 1]) + t for j, t in enumerate(halves(acc))]
    o_ref[...] = jnp.concatenate(out, axis=1).astype(o_ref.dtype)


@jax.jit
def pallas_interleave_layers__sliding_block_cached__mixer_channel_mlp__decode_kernel(
    A_x, A_k_cache, A_v_cache, A_wq, A_wo, B_x, B_w1, B_b1, B_w2, B_b2
):
    Sk = A_k_cache.shape[2]
    assert A_x.shape == (B, 1, D) and A_k_cache.shape == (B, G, Sk, DH) and B_w1.shape == (D, F)
    assert min(4096, max(256, Sk // 4)) == W and Sk % 128 == 0
    wq, wo, w1, w2 = (_tile_view(w) for w in (A_wq, A_wo, B_w1, B_w2))
    w1 = w1.reshape(-1, 16, 128)
    out = pl.pallas_call(
        _kernel,
        out_shape=jax.ShapeDtypeStruct((B, D), A_x.dtype),
        in_specs=[pl.BlockSpec(memory_space=pl.ANY)] * 10,
        scratch_shapes=[
            pltpu.VMEM((B, D), BF),
            pltpu.VMEM((B, G, W, DH), BF),
            pltpu.VMEM((B, G, W, DH), BF),
            pltpu.VMEM(wq.shape, BF),
            pltpu.VMEM(wo.shape, BF),
            pltpu.VMEM(w1.shape, BF),
            pltpu.VMEM((NF, 128), BF),
            pltpu.VMEM((ND, 128), BF),
            pltpu.VMEM((B, G, W // 128, DH, 128), BF),
            pltpu.VMEM((G, (REP + 1) * B, DH), F32),
            pltpu.VMEM((G, (REP + 1) * B, DH), F32),
            pltpu.VMEM((NQ * 8, 128), F32),
            pltpu.VMEM((NF * 8, 128), F32),
            pltpu.VMEM((NQ, 2, 32, 128), BF),
            pltpu.VMEM((len(THIN), 16, 128), BF),
            pltpu.VMEM((NF * 8, 128), F32),
            pltpu.SemaphoreType.DMA((8 + len(PIECES),)),
        ] + [
            pltpu.VMEM((len(kts), 128, 128) if c1 - c0 == 1
                       else (8 * len(kts), 2, (c1 - c0) // 2, 16, 128), BF)
            for kts, c0, c1 in PIECES
        ],
        compiler_params=pltpu.CompilerParams(
            vmem_limit_bytes=100 * 1024 * 1024, disable_semaphore_checks=True),
    )(A_x.reshape(B, D), A_k_cache, A_v_cache, wq, wo, w1, B_b1.reshape(NF, 128),
      w2, B_w2, B_b2.reshape(ND, 128))
    return out.reshape(A_x.shape)
```
